```python
import os as _os
_os.environ.setdefault("JAX_PLATFORMS", "cpu")
import jax
import jax.numpy as jnp

def _softmax(x, axis=-1):
    return jax.nn.softmax(x, axis=axis)
def _gelu(x):
    return jax.nn.gelu(x, approximate=True)
def _silu(x):
    return jax.nn.silu(x)
def _sigmoid(x):
    return jax.nn.sigmoid(x)
def _layernorm(x, axis=-1, eps=1e-5):
    m = jnp.mean(x, axis=axis, keepdims=True)
    v = jnp.var(x, axis=axis, keepdims=True)
    return (x - m) / jnp.sqrt(v + eps)
def _scatter_add(tgt, idx, src, axis=0):
    return tgt.at[idx].add(src)
def _segment_sum(src, seg, n):
    return jax.ops.segment_sum(src, seg, n)
class _Rng:
    def __init__(self, key):
        self._k = key
    def _next(self):
        self._k, sub = jax.random.split(self._k)
        return sub
    def normal(self, shape):
        return jax.random.normal(self._next(), shape, dtype=jnp.bfloat16)
    def randint(self, lo, hi, shape):
        return jax.random.randint(self._next(), shape, lo, hi, dtype=jnp.int32)
    def uniform(self, shape, lo=0.0, hi=1.0):
        return jax.random.uniform(self._next(), shape, jnp.bfloat16, lo, hi)
    def permutation(self, n):
        return jax.random.permutation(self._next(), n)


kernel_name = 'parallel_sum__softmax_full_mha__glu_gated_swiglu__prompt'

def setup_inputs():
    _rng = _Rng(jax.random.key(int.from_bytes(__import__("os").urandom(4), "little")))
    _w = (lambda a: (lambda t: t.astype(jnp.bfloat16) if jnp.issubdtype(t.dtype, jnp.floating) else t)(jnp.asarray(a)))
    def _A_setup():
        B, S, D = 1, 2048, 448
        return {
            "x": _w((lambda *s: _rng.normal(s) * 0.05)(B, S, D)),
            "wqkv": _w((lambda *s: _rng.normal(s) * 0.05)(D, 3 * D)),
            "wo": _w((lambda *s: _rng.normal(s) * 0.05)(D, D)),
        }
    _A_in = _A_setup()

    def _B_setup():
        B, S, D, F = 1, 2048, 448, 1792
        return {
            "x": _w((lambda *s: _rng.normal(s) * 0.05)(B, S, D)),
            "w1": _w((lambda *s: _rng.normal(s) * 0.05)(D, F) * (2.0 / D) ** 0.5),
            "w3": _w((lambda *s: _rng.normal(s) * 0.05)(D, F) * (2.0 / D) ** 0.5),
            "w2": _w((lambda *s: _rng.normal(s) * 0.05)(F, D) * (2.0 / F) ** 0.5),
        }
    _B_in = _B_setup()

    return {
        "A_x": _A_in["x"],
        "A_wqkv": _A_in["wqkv"],
        "A_wo": _A_in["wo"],
        "B_x": _B_in["x"],
        "B_w1": _B_in["w1"],
        "B_w3": _B_in["w3"],
        "B_w2": _B_in["w2"],
    }

def reference(A_x, A_wqkv, A_wo, B_x, B_w1, B_w3, B_w2):
    def _A_ref(x, wqkv, wo):
        B, S, D = x.shape
        H = 16; Dh = D // H
        qkv = (lambda x, *d: x.transpose(*d))((x @ wqkv).reshape(B, S, 3, H, Dh), 2, 0, 3, 1, 4)
        q, k, v = qkv[0], qkv[1], qkv[2]
        scale = Dh ** -0.5
        scores = jnp.einsum("bhqd,bhkd->bhqk", q, k) * scale
        p = _softmax(scores, axis=-1)
        o = jnp.einsum("bhqk,bhkd->bhqd", p, v)
        return (lambda x, *d: x.transpose(*d))(o, 0, 2, 1, 3).reshape(B, S, D) @ wo

    def _B_ref(x, w1, w3, w2):
        gate = jnp.einsum("bsd,df->bsf", x, w1)
        up = jnp.einsum("bsd,df->bsf", x, w3)
        h = _silu(gate) * up
        out = jnp.einsum("bsf,fd->bsd", h, w2)
        return out

    x = A_x
    xn = _layernorm(x, axis=-1)
    return x + _A_ref(xn, A_wqkv, A_wo) + _B_ref(xn, B_w1, B_w3, B_w2)
```

```python
import functools
import math
import jax
import jax.numpy as jnp
from jax import lax
from jax.experimental import pallas as pl
from jax.experimental.pallas import tpu as pltpu

f32 = jnp.float32
bf16 = jnp.bfloat16
u32 = jnp.uint32
H = 16
EPS = 1e-5


def _win(h, dh):
    start = (h * dh) // 8 * 8
    return start, h * dh - start


def _pk(x):
    return pltpu.bitcast(x, u32)


def _up(x):
    return pltpu.bitcast(x, bf16)


def build(BQ=512, NS=4, CH=128, TB=512, TC=512, FCH=448, flags=None, name="fused"):
    def kernel(xT_hbm, wqkv_hbm, wo_hbm, w1_hbm, w3_hbm, w2T_hbm, oT_hbm,
               x_v, wqkv_v, wo_v, w1_v, w3_v, w2T_v, o_v,
               xn_s, wqkvT_s, w1T_s, w3T_s, woT_s, q_s, k_s, v_s, a_s, h_s, sa, sb,
               xsem, wsem, osem):
        D, S = x_v.shape
        F = w1_v.shape[1]
        dh = D // H
        NC = S // CH
        NQ = S // BQ
        qscale = dh ** -0.5 * math.log2(math.e)

        x_cp = [pltpu.make_async_copy(xT_hbm.at[:, t * TB:(t + 1) * TB], x_v.at[:, t * TB:(t + 1) * TB], xsem.at[t])
                for t in range(S // TB)]
        w_cp = [pltpu.make_async_copy(s, d, wsem.at[n]) for n, (s, d) in enumerate(
            [(wqkv_hbm, wqkv_v), (w1_hbm, w1_v), (w3_hbm, w3_v), (wo_hbm, wo_v), (w2T_hbm, w2T_v)])]
        x_cp[0].start()
        w_cp[0].start()
        for c in x_cp[1:]:
            c.start()
        for c in w_cp[1:]:
            c.start()

        row = lax.broadcasted_iota(jnp.int32, (32, TB), 0)
        for t in range(S // TB):
            sl = slice(t * TB, (t + 1) * TB)
            x_cp[t].wait()
            x = x_v[:, sl].astype(f32)
            m = jnp.sum(x, axis=0, keepdims=True) * (1.0 / D)
            xc = x - m
            v = jnp.sum(xc * xc, axis=0, keepdims=True) * (1.0 / D)
            xn = (xc * lax.rsqrt(v + EPS)).astype(bf16)
            xn_s[:, sl] = _pk(xn)
            if t == 0:
                w_cp[0].wait()
                wqkvT_s[...] = _pk(wqkv_v[...].T)
            qkv = jnp.dot(_up(wqkvT_s[...]), xn, preferred_element_type=f32)
            ks = []
            for h in range(H):
                st, off = _win(h, dh)
                valid = (row >= off) & (row < off + dh)
                q = jnp.where(valid, qkv[st:st + 32] * qscale, 0.0)
                vv = jnp.where(valid, qkv[2 * D + st:2 * D + st + 32], 1.0)
                q_s[h, :, sl] = _pk(q.astype(bf16))
                v_s[h, :, sl] = _pk(vv.astype(bf16))
                ks.append(qkv[D + st:D + st + 32])
                if h % 4 == 3:
                    kk = jnp.concatenate(ks, axis=0).astype(bf16)
                    k_s[h // 4, t * TB // 2:(t + 1) * TB // 2, :] = _pk(kk.T)
                    ks = []
            if t == S // TB - 2:
                w_cp[1].wait()
                w1T_s[...] = _pk(w1_v[...].T)
            if t == S // TB - 1:
                w_cp[2].wait()
                w3T_s[...] = _pk(w3_v[...].T)
                w_cp[3].wait()
                woT_s[...] = _pk(wo_v[...].T)

        row8 = lax.broadcasted_iota(jnp.int32, (8, BQ), 0)

        def s_chunk(g, u, q0, c, s_w, mx):
            q = _up(q_s[4 * g + u, :, pl.ds(q0, BQ)])
            if u > 0:
                q = jnp.concatenate([jnp.zeros((32 * u, BQ), bf16), q], axis=0)
            kk = _up(k_s[g, c * CH // 2:(c + 1) * CH // 2, :])[:, :32 * (u + 1)]
            s = jnp.dot(kk, q, preferred_element_type=f32)
            s_w[c * CH:(c + 1) * CH, :] = s
            cm = jnp.max(s.reshape(CH // 8, 8, BQ), axis=0)
            return cm if mx is None else jnp.maximum(mx, cm)

        def pv_chunk(h, c, s_r, z, m, acc):
            sp = s_r[pl.ds(z + c * CH, CH), :].reshape(CH // 8, 8, BQ)
            p = jnp.exp2(sp - m[None]).reshape(CH, BQ).astype(bf16)
            d = jnp.dot(_up(v_s[h, :, c * CH:(c + 1) * CH]), p, preferred_element_type=f32)
            return d if acc is None else acc + d

        def fin_max(mx):
            return jnp.broadcast_to(jnp.max(mx, axis=0, keepdims=True), (8, BQ))

        def group(it, z, m, n_groups, last):
            for gg in range(n_groups):
                gi = it * n_groups + gg
                g = gi % 4
                q0 = (gi // 4) * BQ
                gn = (gi + 1) % 4
                q0n = ((gi + 1) // 4) * BQ
                if not isinstance(gi, int):
                    q0 = pl.multiple_of(q0, BQ)
                    q0n = pl.multiple_of(q0n, BQ)
                outs = []
                for u in range(4):
                    s_r, s_w = (sa, sb) if u % 2 == 0 else (sb, sa)
                    mx = acc = None
                    skip = last and gg == n_groups - 1 and u == 3
                    for c in range(NC):
                        if u < 3:
                            mx = s_chunk(g, u + 1, q0, c, s_w, mx)
                        elif not skip:
                            mx = s_chunk(gn, 0, q0n, c, s_w, mx)
                        acc = pv_chunk(4 * g + u, c, s_r, z, m, acc)
                    if not skip:
                        m = fin_max(mx)
                    l = acc[31:32] if u % 2 == 0 else acc[0:1]
                    outs.append(acc * (1.0 / l))
                parts = []
                for u in (0, 2):
                    e, o = outs[u], outs[u + 1]
                    parts += [e[0:24], jnp.where(row8 < 4, e[24:32], o[0:8]), o[8:32]]
                r0 = g * (2 * dh)
                if not isinstance(gi, int):
                    r0 = pl.multiple_of(r0, 8)
                a_s[pl.ds(r0, 2 * dh), pl.ds(q0, BQ)] = _pk(jnp.concatenate(parts, axis=0).astype(bf16))
            return m

        mx = None
        for c in range(NC):
            mx = s_chunk(0, 0, 0, c, sa, mx)
        m0 = fin_max(mx)
        NG = NS // 4
        n_it = NQ * 4 // NG

        def body(it, carry):
            z = pl.multiple_of((it // 4096) * 8, 8)
            return group(it, z, carry[0], NG, False), z

        m, z = lax.fori_loop(0, n_it - 1, body, (m0, jnp.int32(0)))
        group(n_it - 1, pl.multiple_of(z, 8), m, NG, True)

        w_cp[4].wait()

        def o_cp(t):
            c0 = pl.multiple_of(t * TC, TC)
            return pltpu.make_async_copy(o_v.at[:, pl.ds(c0, TC)], oT_hbm.at[:, pl.ds(c0, TC)], osem.at[t])

        def cbody(t, carry):
            c0 = pl.multiple_of(t * TC, TC)
            xn = _up(xn_s[:, pl.ds(c0, TC)])
            for j in range(F // FCH):
                r = slice(j * FCH // 2, (j + 1) * FCH // 2)
                g = jnp.dot(_up(w1T_s[r, :]), xn, preferred_element_type=f32)
                up = jnp.dot(_up(w3T_s[r, :]), xn, preferred_element_type=f32)
                h_s[r, :] = _pk((g * jax.nn.sigmoid(g) * up).astype(bf16))
            y = jnp.dot(_up(woT_s[...]), _up(a_s[:, pl.ds(c0, TC)]), preferred_element_type=f32)
            y = y + jnp.dot(w2T_v[...], _up(h_s[...]), preferred_element_type=f32)
            o_v[:, pl.ds(c0, TC)] = (x_v[:, pl.ds(c0, TC)].astype(f32) + y).astype(bf16)
            o_cp(t).start()
            return carry

        lax.fori_loop(0, S // TC, cbody, 0)
        for t in range(S // TC):
            o_cp(t).wait()

    def fn(A_x, A_wqkv, A_wo, B_x, B_w1, B_w3, B_w2):
        B, S, D = A_x.shape
        F = B_w1.shape[1]
        xT = A_x.reshape(S, D).T
        args = (xT, A_wqkv, A_wo, B_w1, B_w3, B_w2.T)
        V = pltpu.VMEM
        oT = pl.pallas_call(
            kernel, name=name,
            in_specs=[pl.BlockSpec(memory_space=pl.ANY)] * len(args),
            out_specs=pl.BlockSpec(memory_space=pl.ANY),
            out_shape=jax.ShapeDtypeStruct((D, S), bf16),
            scratch_shapes=[V(a.shape, bf16) for a in args] + [
                V((D, S), bf16),
                V((D // 2, S), u32), V((3 * D // 2, D), u32), V((F // 2, D), u32), V((F // 2, D), u32),
                V((D // 2, D), u32), V((H, 16, S), u32), V((H // 4, S // 2, 128), u32), V((H, 16, S), u32),
                V((D // 2, S), u32), V((F // 2, TC), u32), V((S, BQ), f32), V((S, BQ), f32),
                pltpu.SemaphoreType.DMA((S // TB,)), pltpu.SemaphoreType.DMA((5,)),
                pltpu.SemaphoreType.DMA((S // TC,))],
            compiler_params=pltpu.CompilerParams(vmem_limit_bytes=100 * 2**20, flags=flags),
        )(*args)
        return oT.T.reshape(B, S, D)
    return fn


@jax.jit
def pallas_parallel_sum__softmax_full_mha__glu_gated_swiglu__prompt_kernel(
    A_x: jax.Array,
    A_wqkv: jax.Array,
    A_wo: jax.Array,
    B_x: jax.Array,
    B_w1: jax.Array,
    B_w3: jax.Array,
    B_w2: jax.Array,
):
    return build()(A_x, A_wqkv, A_wo, B_x, B_w1, B_w3, B_w2)
```

```python
import functools
import math

import jax
import jax.numpy as jnp
import numpy as np
from jax import lax
from jax.experimental import pallas as pl
from jax.experimental.pallas import tpu as pltpu

f32 = jnp.float32
bf16 = jnp.bfloat16
u32 = jnp.uint32
P = functools.partial

S, D, F, H = 2048, 448, 1792, 16
EPS = 1e-5
LOG2E = math.log2(math.e)

DH = D // H
D2, D4, D8, F4 = D // 2, D // 4, D // 8, F // 4
T = 512
NT = S // T
NC = S // 128
NG = 14
NV = 16 * NG
NM = S - NV
NW = -(-NV // 128)
DSTEP = 7
R = 64
AX = 512 - F4
AR = (D - 4 * AX) // 2
HEADROOM = 30.0

O_W13 = 32
O_W2 = O_W13 + 49 * (F4 // 2)
W_END = O_W2 + 53 * D4 + 80
O_XE = 32
X_END = O_XE + NT * 28 * D8
A_P = 32
A_K = A_P + 32
A_KT = A_K + S // 2
A_QT = A_KT + DH * NV + 16
A_KR = A_QT + NC * (DH + 1) * 8 + 16
A_END = A_KR + NW * (H // 2) * 64


def _pk(x):
    return pltpu.bitcast(x.astype(bf16), u32)


def _up(x):
    return pltpu.bitcast(x, bf16)


def _raw(x):
    return pltpu.bitcast(x, u32)


def _flt(x):
    return pltpu.bitcast(x, f32)


def _dot(a, b):
    return jnp.dot(a, b, preferred_element_type=f32)


def _cat(xs, axis):
    return jnp.concatenate(xs, axis=axis)


def _part(j, n):
    return slice(j * n, (j + 1) * n) if isinstance(j, int) else pl.ds(pl.multiple_of(j * n, n), n)


ENC_A = (((1, 0), (1, 3)), ((1, 2), (1, 3)), ((1, 0),), ((1, 3),), ((1, 0), (1, 1)), ((1, 2), (-1, 0)),
         ((1, 1), (-1, 3)))
ENC_B = (((1, 0), (1, 3)), ((1, 0),), ((1, 1), (-1, 3)), ((1, 2), (-1, 0)), ((1, 3),), ((1, 0), (1, 1)),
         ((1, 2), (1, 3)))
FLIP = (0, 1, 0, 0, 1, 1, 1)


def _comb(terms, get):
    x = get(terms[0][1])
    if len(terms) == 1:
        return x
    y = get(terms[1][1])
    return x + y if terms[1][0] > 0 else x - y


def _enc7(enc, r, get):
    o = [_comb(enc[r], lambda q: get(2 * (q // 2) + p // 2, 2 * (q % 2) + p % 2)) for p in range(4)]
    flip = FLIP[r] if enc is ENC_B else 0
    return [_comb(enc[s], lambda p: o[p ^ flip]) for s in range(7)]


def _dec(m):
    return [m[0] + m[3] - m[4] + m[6], m[2] + m[4], m[1] + m[3], m[0] - m[1] + m[2] + m[5]]


def _dec2(prod, extra=None):
    inner = [_dec([prod(r, s) for s in range(7)]) for r in range(7)]
    inner = [[m[p ^ f] for p in range(4)] for m, f in zip(inner, FLIP)]
    if extra:
        inner = [[x + y for x, y in zip(*e)] for e in zip(inner, extra)]
    out = [[None] * 4 for _ in range(4)]
    for i in range(2):
        for j in range(2):
            out[i][j], out[i][j + 2], out[i + 2][j], out[i + 2][j + 2] = _dec([m[2 * i + j] for m in inner])
    return out


class _Pace:
    def __init__(self, jobs, ticks, gate, tie, lag, lead=0):
        self.jobs, self.ticks, self.gate, self.tie, self.lag, self.lead = jobs, ticks, gate, tie, lag, lead
        self.pos, self.done, self.hist, self.last, self.later = 0, 0, [], -1, []

    def restart(self, jobs, ticks, gate, tie):
        self.run(len(self.jobs))
        self.jobs, self.ticks, self.gate, self.tie, self.lead, self.done = jobs, ticks, gate, tie, self.pos, 0

    def run(self, upto):
        while self.done < min(upto, len(self.jobs)):
            k = min(self.pos - self.lag, len(self.hist) - 1)
            if k > self.last:
                for ref in self.gate:
                    ref[:8, :128] = _raw(self.hist[k])
                self.last = k
            self.jobs[self.done]()
            self.done += 1

    def tick(self):
        done = self.done
        self.run((self.pos - self.lead) * len(self.jobs) // self.ticks)
        self.pos += 1
        due = [job for n, job in self.later if n == 0]
        self.later = [(n - 1, job) for n, job in self.later if n > 0]
        for job in due:
            job()
        return self.done > done or bool(due)

    def lhs(self, ref, o, n, lanes, tied=False):
        out = []
        for r in range(o, o + n, 8):
            ran = self.tick()
            x = ref[r:r + 8, lanes]
            for tie in self.tie if ran and not tied else []:
                x = x | tie()[16:24, :x.shape[1]]
            out.append(x)
        return _cat(out, 0)

    def result(self, y):
        self.hist += [y[r + 8:r + 16, -128:] for r in range(0, y.shape[0], 16)]

    def finish(self):
        self.run(len(self.jobs))
        for _, job in self.later:
            job()
        self.later = []


def _merge(main, *lists, skip=0):
    def both(n):
        for lst in lists:
            for job in lst[max(n - skip, 0) * len(lst) // (len(main) - skip):
                           max(n + 1 - skip, 0) * len(lst) // (len(main) - skip)]:
                job()
        main[n]()
    return [P(both, n) for n in range(len(main))]


def _kernel(xT_hbm, wqkv_hbm, wo_hbm, w1_hbm, w3_hbm, w2T_hbm, oT_hbm,
            x_v, wqkv_v, wo_v, w13_v, w2T_v, o_v,
            ew_s, ex_s, xf_s, wt_s, wd_s, xn_s, wqkvT_s, h_s, q_s, qf_s, k_s, v_s, a_s, chk_s, p_s, aa0, aa1,
            xsem, wsem, osem):
    x_cuts = (0, 512, 1280, S)
    x_cp = [pltpu.make_async_copy(xT_hbm.at[:, a:b], x_v.at[:, a:b], xsem.at[n])
            for n, (a, b) in enumerate(zip(x_cuts, x_cuts[1:]))]
    w_cuts = (0, 128, 512, 3 * D)
    w_cp = [pltpu.make_async_copy(src, dst, wsem.at[n]) for n, (src, dst) in enumerate(
        [(wqkv_hbm.at[:, a:b], wqkv_v.at[:, a:b]) for a, b in zip(w_cuts, w_cuts[1:])]
        + [(w1_hbm, w13_v.at[0]), (wo_hbm, wo_v), (w2T_hbm, w2T_v), (w3_hbm, w13_v.at[1])])]
    x_cp[0].start()
    w_cp[0].start()
    w_cp[1].start()

    zero = [lax.fori_loop(0, 2, lambda i, c: (c + i) >> 12, np.int32(0))]
    views = [0]

    def view(ref, start=0, size=None):
        views[0] += 1
        return ref.at[pl.ds(pl.multiple_of(zero[0] * (32 * views[0]) + start, 32), size or ref.shape[0])]

    row = lax.broadcasted_iota(jnp.int32, (32, 256), 0)

    def window(y, h, first, rest):
        off = 4 * (h % 2)
        w = y[h * DH - off:h * DH - off + 32]
        b = slice(0, 8) if off else slice(24, 32)
        fill = jnp.where(row[b] == (0 if off else DH), first, rest)
        e = jnp.where((row[b] >= off) & (row[b] < off + DH), w[b], fill)
        return _cat([e, w[8:]] if off else [w[:24], e], 0)

    def layernorm(jp):
        stat = {}

        def rows(c):
            return view(x_v)[_part(c, 32), _part(jp, 256)].astype(f32)

        def total(x, n, c):
            x = x[0:8] + x[8:16] + (x[16:24] + x[24:32])
            stat[n] = x if c == 0 else stat[n] + x
            if c == D // 32 - 1:
                stat[n] = jnp.sum(stat[n], axis=0, keepdims=True) * (1.0 / D)
            xf_s[8:16, :] = _raw(jnp.broadcast_to(stat[n], (8, 256)))

        def mean(c):
            total(rows(c), 0, c)

        def var(c):
            xc = rows(c) - stat[0]
            total(xc * xc, 1, c)

        def put(c):
            xn = (rows(c) - stat[0]) * lax.rsqrt(stat[1] + EPS)
            xf_s[32 + jp * D + c * 32:32 + jp * D + (c + 1) * 32, :] = _raw(xn)
            xn_s[_part(c, 16), _part(jp, 256)] = _pk(xn)
        return [P(f, c) for f in (mean, var, put) for c in range(D // 32)]

    def put_q(jp, q):
        qf_s[:, :2 * DH, _part(jp, 256)] = (q * (DH ** -0.5 * LOG2E)).reshape(H // 2, 2 * DH, 256)

    def put_qk(jp, g, k):
        sl = _part(jp, 256)

        def head(n):
            h = 4 * g + n
            q = qf_s[h // 2, :2 * DH, sl]
            own = jnp.sum(window(q * k[_part(n // 2, 2 * DH)], h % 2, 0.0, 0.0), axis=0, keepdims=True)
            shift = (-HEADROOM - own).astype(bf16).astype(f32)
            qf_s[h // 2, 2 * DH + h % 2:2 * DH + h % 2 + 1, sl] = shift
            q_s[_part(h, 16), sl] = _pk(window(q, h % 2, shift, 0.0))
            ex_s[8:16, :] = q_s[_part(2 * h + 1 - h % 2, 8), sl]

        def keys(n):
            kT = _raw(_cat([window(k, h, 1.0, 0.0) for h in range(4)], 0)[:, _part(n, 128)].astype(bf16).T)
            k_s[g, _part((jp + 7) % 8 * 2 + n, 64), :] = kT
            ex_s[8:16, :128] = kT[-8:]

        def key_rows(w, n):
            o = A_KR + (w * (H // 2) + 2 * g + n) * 64
            for ref in (aa0, aa1):
                ref[o:o + 2 * DH, :] = _raw(pltpu.roll(k, NV % 256, 1)[_part(n, 2 * DH), _part(w, 128)])
        return ([(10 + 2 * n, P(head, n)) for n in range(4)] + [(30 + 6 * n, P(keys, n)) for n in range(2)]
                + [(22 + 2 * n + w, P(key_rows, w, n)) for n in range(2) for w in range(NW) if jp == 0])

    def project(part, jp, pace, half=0):
        ys = []

        def rhs(n):
            return _up(view(xn_s).at[:, _part(half + jp // 4, S // 2)][:, _part(jp % 4 * 2 + n, 128)])
        xn = [rhs(n) for n in range(2)] if part == 0 else None
        for g in range(4):
            o = part * D2 + g * D8
            y = []
            for n in range(2):
                src = view(wqkvT_s)
                lhs = _cat([pace.lhs(src, o, D8, slice(0, 128)), src[o:o + D8, 128:]], 1)
                y.append(_dot(_up(lhs), xn[n] if xn else rhs(n)))
                pace.result(y[-1])
            ys.append(_cat(y, 1))
            if part == 1:
                pace.later += put_qk(jp, g, ys[-1])
            if part == 2:
                for n in range(4):
                    v_s[_part(4 * g + n, 16), _part((4 * half + jp + 7) & 7, 256)] = _pk(window(ys[-1], n, 1.0, 1.0))
        return _cat(ys, 0)

    def enc_x(t, c, r):
        src = view(xf_s)

        def get(i, j):
            o = 32 + (2 * t + j // 2) * D + i * D4 + c * 16
            return _flt(src[o:o + 16, _part(j % 2, 128)])
        e = _enc7(ENC_B, r, get)
        for p in range(4):
            o = O_XE + ((t * 7 + r) * 4 + p) * D8 + c * 8
            ex_s[o:o + 8, :] = _pk(_cat([e[2 * p], e[min(2 * p + 1, 6)]], 1))

    def enc_w(src, where, dst, stride, o, r):
        src = view(src)
        for s, e in enumerate(_enc7(ENC_A, r, lambda i, j: _up(
                _cat([src[a:a + 8, :] for a in where(i, j)], 1)).astype(f32))):
            dst[o + (7 * r + s) * stride:o + (7 * r + s) * stride + 8, :] = _pk(e)

    def enc_w13(dst, n, r):
        enc_w(wt_s, lambda i, j: [32 + j * (F // 2) + a + (192 * i + 16 * n if n < 12 else 576 + 32 * i + 16 * n)
                                  for a in (0, 8)], dst, F4 // 2, n * 16, r)

    def enc_w2(dst, c, r):
        enc_w(wd_s, lambda i, j: [32 + (2 * j + a) * D2 + i * D8 + c * 8 for a in range(2)], dst, D4, c * 8, r)

    def enc_wo(dst, m, c):
        src = view(wd_s).at[pl.ds(pl.multiple_of(32 + 4 * D + m * D8, 8), D - D8)]
        q = [_up(src[o + c * 8:o + c * 8 + 8, :]).astype(f32) for o in (0, D2, D4, D2 + D4)]
        for p in range(4):
            o = (49 + p) * D4 + c * 8
            dst[o:o + 8, :] = _pk(_cat([_comb(ENC_A[r], lambda n: q[n]) for r in (2 * p, min(2 * p + 1, 6))], 1))

    def wo_t(r0, n):
        w = _cat([wo_v[r0:r0 + n, :], jnp.zeros((n, 512 - D), bf16)], 1)
        if n % 128:
            w = _cat([w, jnp.zeros((-n % 128, 512), bf16)], 0)
        return _raw(w.T)[:D2]

    def lay_out_weights(m):
        woT = wo_t(0, 4 * AX)
        for n in range(2):
            wd_s[32 + 4 * D + n * D2:32 + 4 * D + (n + 1) * D2, :] = wo_t(4 * AX + n * AR, AR)
        lane = lax.broadcasted_iota(jnp.int32, (D2, 128), 1)
        for j in range(4):
            o = 32 + 2 * j * D2
            wd_s[o:o + D2, :] = _raw(w2T_v[:, pl.ds(pl.multiple_of(384 * j + 256 * m, 128), 128)])
            b = _raw(w2T_v[:, _part(12 + j // 2, 128)])
            wo = woT[:, _part(j // 2, 128)]
            b = jnp.where(lane < 64, b, wo) if j % 2 == 0 else pltpu.roll(jnp.where(lane < 64, wo, b), 64, 1)
            wd_s[o + D2:o + D, :] = jnp.where(m == 0, _raw(w2T_v[:, _part(3 * j + 1, 128)]), b)
        for j in range(4):
            w = _cat([w13_v[m, _part(j, D4), :], jnp.zeros((128 - D4, F), bf16)], 0)
            wt_s[32 + j * (F // 2):32 + (j + 1) * (F // 2), :] = _raw(w.T)

    def key_table(dst, src, par, ahead):
        val = {}

        def start(d, w):
            r, n = par * DH + d, min(128, NV - 128 * w)
            o = A_KR + w * (H // 2) * 64 + r // 8 * 8
            val[d, w] = jnp.broadcast_to(src()[o:o + 8, :n][r % 8:r % 8 + 1], (128, n)).T

        def put(d, g):
            o = A_KT + (g * DH + d) * 16
            dst[o:o + 16, :] = val[d, g // 8][_part(g % 8, 16)]
        puts = [(d, g) for d in range(DH) for g in range(NG)]
        jobs = []
        for n in range(len(puts) + ahead):
            if n < len(puts) and puts[n][1] % 8 == 0:
                jobs.append(P(start, puts[n][0], puts[n][1] // 8))
            if n >= ahead:
                jobs.append(P(put, *puts[n - ahead]))
        return jobs

    def query_table(dst, src, par, pairs):
        def put(j, d):
            r = par * DH + d if d < DH else 2 * DH + par
            dst[_part(j * (DH + 1) + d, 16), :] = _raw(_cat(
                [jnp.broadcast_to(src[r:r + 1, _part(2 * j + n, 128)], (8, 128)) for n in range(2)], 0))
        return [P(put, j, d) for j in range(pairs) for d in range(DH + 1)]

    def head_k(h, rows):
        return pltpu.roll(k_s[h >> 2, rows, :], (-h & 3) * 32, 1)

    def put_k(dst, h, r):
        dst[A_K + r:A_K + r + 8, :] = head_k(h, slice(r, r + 8))

    def head_rows(ref, h):
        return ref.at[_part(h, 16)]

    def put_a(h, par, sl, acc):
        inv = pltpu.reciprocal(acc[0:1] if par else acc[31:32], approx=True)
        a_s[h >> 1, _part(par, DH), sl] = (acc * inv)[4 * par:4 * par + DH]
        return inv

    def weigh(h, par, t, j, c, acc, pace, dst):
        p = p_s.at[:, _part(t, T)][_part(par * 4 + c, 256), _part(j, 128)]
        src = head_rows(view(v_s), h)
        v = _cat([pace.lhs(src, 0, 16, _part(4 * c, 128)), src[:, c * 512 + 128:(c + 1) * 512]], 1)
        d = _dot(_up(v), _up(p))
        acc = d if c == 0 else d + acc
        pace.result(acc)
        if c == 3:
            inv = put_a(dst, par, _part(4 * t + j, 128), acc)
            a = jnp.abs(acc)
            chk_s[:8] += a[0:8] + a[8:16] + (a[16:24] + a[24:32]) + inv * 2.0 ** 80
        return acc

    def head_step(h, par):
        cur, oth = (aa0, aa1) if par == 0 else (aa1, aa0)
        hn = jnp.minimum(h + 1, H - 1)
        part = []

        def unit(jp, g, d0):
            src = view(oth)
            oq, ok = A_QT + jp * (DH + 1) * 16, A_KT + g * DH * 16
            if d0 == 0:
                q = _flt(src[oq + DH * 16:oq + (DH + 1) * 16, :])
                part[:] = [_cat([q[o:o + 8]] * 2, 0) for o in (0, 8)]
            k = _flt(src[ok + d0 * 16:ok + (d0 + DSTEP) * 16, :])
            q = _flt(src[oq + d0 * 16:oq + (d0 + DSTEP) * 16, :])
            for o in range(0, DSTEP * 16, 16):
                part[:] = [a + k[o:o + 16] * _cat([q[o + n:o + n + 8]] * 2, 0) for a, n in zip(part, (0, 8))]
            cur[A_P:A_P + 32, :] = _raw(_cat(part, 0))
            if d0 + DSTEP == DH:
                o = (par * S + NM) // 2 + g * 8
                p_s[o:o + 8, _part(jp, 256)] = _pk(jnp.exp2(_cat(part, 1)))

        jobs = _merge([P(unit, jp, g, d0) for jp in range(NC // 2) for g in range(NG) for d0 in range(0, DH, DSTEP)],
                      key_table(cur, P(view, oth, (hn >> 1) * 64, A_END - (H // 2 - 1) * 64), 1 - par, 12),
                      query_table(cur.at[A_QT:], qf_s.at[hn >> 1], 1 - par, NC // 2),
                      [P(put_k, oth, hn, r) for r in range(0, NM // 2, 8)], skip=2)
        pace = _Pace(jobs, NT * (NM // 16 + 2 * NC) - 6, [oth], [P(view, cur)], 13, 8)
        acc = None
        for t in range(NT):
            for c in range(NC):
                a, b = NM // 16 * c // NC * 8, NM // 16 * (c + 1) // NC * 8
                last = t == NT - 1 and c == NC - 1
                if last:
                    weigh(h - 1, 1 - par, t, c // 4, c % 4, acc, pace, h - 1)
                k = pace.lhs(view(cur) if t + c else cur, A_K + a, b - a, slice(0, 32), tied=True)
                s = _dot(_up(k), _up(head_rows(q_s, h)[:, _part(t, T)]))
                pace.result(s)
                if not last:
                    acc = weigh(h - 1, 1 - par, t, c // 4, c % 4, acc, pace, h - 1)
                p_s[par * S // 2 + a:par * S // 2 + b, _part(t, T)] = _pk(jnp.exp2(s))
        pace.finish()

    def exact_softmax():
        @pl.loop(0, H * NC)
        def _(n):
            h, sl = n // NC, _part(n % NC, 128)
            q = _up(head_rows(q_s, h)[:, sl]).astype(f32)
            q = jnp.where(row[:, :128] == (1 - h % 2) * DH, 0.0, q).astype(bf16)

            def scores(c, m):
                s = _dot(_up(head_k(h, _part(c, 256))[:, :32]), q)
                h_s[_part(c, 512), :] = s
                return jnp.maximum(m, jnp.max(s, axis=0, keepdims=True))
            m = lax.fori_loop(0, 4, scores, jnp.full((1, 128), -jnp.inf, f32))
            acc = lax.fori_loop(0, 4, lambda c, acc: acc + _dot(
                _up(head_rows(v_s, h)[:, _part(c, 512)]), jnp.exp2(h_s[_part(c, 512), :] - m).astype(bf16)),
                jnp.zeros((32, 128), f32))
            for par in range(2):
                @pl.when(h % 2 == par)
                def _():
                    put_a(h, par, sl, acc)

    def a_rows(src, r0, r1, sl):
        n = 2 * DH
        return _cat([src[g, max(r0 - g * n, 0):min(r1 - g * n, n), sl] for g in range(r0 // n, -(-r1 // n))], 0)

    def output_block(trip, t):
        zero[0] = t >> 12
        last_head = [0, None]
        for c in range(F4 // R):
            xe = view(ex_s, t * 28 * D8, O_XE + 28 * D8)

            def up(r, s):
                if (49 * c + 7 * r + s) % 8 == 4 and last_head[0] < 16:
                    last_head[1] = weigh(H - 1, 1, t, last_head[0] // 4, last_head[0] % 4, last_head[1],
                                         _Pace([], 1, [], [], 0), H - 1 + trip * 2)
                    last_head[0] += 1
                o = O_W13 + (7 * r + s) * (F4 // 2) + c * R // 2
                w = ew_s[o:o + R // 2, :]
                lhs = _cat([w[_part(n // 2 * 2 + m, 8), n % 2 * 128:n % 2 * 128 + D4]
                            for m in range(2) for n in range(R // 16)], 0)
                o = O_XE + (4 * r + s // 2) * D8
                return _dot(_up(lhs), _up(xe[o:o + D8, _part(s % 2, 128)]))
            hid = [[y[:R] * y[R:] * pltpu.reciprocal(1.0 + jnp.exp2(y[:R] * -LOG2E), approx=True) for y in ys]
                   for ys in _dec2(up)]
            for p in range(4):
                for r in range(7):
                    h_s[(4 * r + p) * F4 + c * R:(4 * r + p) * F4 + (c + 1) * R, :] = _comb(
                        ENC_B[r], lambda q: hid[2 * (q // 2) + p // 2][2 * (q % 2) + p % 2])

        av = view(a_s).at[:, :, _part(t, T)]
        extra = []
        for r in range(7):
            e = _comb(ENC_B[r], lambda q: a_rows(av, 4 * AX + q // 2 * AR, 4 * AX + (q // 2 + 1) * AR,
                                                 _part(q % 2, 256)))
            o = O_W2 + (49 + r // 2) * D4
            extra.append([_dot(_up(ew_s[o + p // 2 * D8:o + (p // 2 + 1) * D8, r % 2 * 128:r % 2 * 128 + AR]),
                               e[:, _part(p % 2, 128)].astype(bf16)) for p in range(4)])

        def down(r, s):
            hv, av = view(h_s), view(a_s).at[:, :, _part(t, T)]

            def a_blk(p, q):
                i, j = (2 * (q // 2) + p // 2) ^ 1, 2 * (q % 2) + p % 2
                return a_rows(av, i * AX, (i + 1) * AX, _part(j, 128))
            e = _comb(ENC_B[s], lambda p: _cat([hv[_part(4 * r + (p ^ FLIP[r]), F4), :],
                                                _comb(ENC_B[r], P(a_blk, p ^ FLIP[r]))], 0))
            o = O_W2 + (7 * r + s) * D4
            return _dot(_up(_cat([ew_s[o:o + D8, :], ew_s[o + D8:o + D4, :]], 1)), e.astype(bf16))
        y = _dec2(down, extra)
        for q in (2, 1, 3, 0):
            rows, lanes = _part(q // 2, D2), _part(2 * t + q % 2, 256)
            yq = _cat([_cat(y[q // 2 * 2 + n][_part(q % 2, 2)], 1) for n in range(2)], 0)
            view(o_v)[rows, lanes] = (x_v.at[:, _part(t, T)][rows, _part(q % 2, 256)].astype(f32) + yq).astype(bf16)
            pltpu.make_async_copy(o_v.at[rows, lanes], oT_hbm.at[rows, lanes], osem).start()

    x_cp[0].wait()
    x_cp[1].start()
    w_cp[0].wait()
    wqkvT_s[:64, :] = _raw(wqkv_v[:, :128].T)
    for job in layernorm(0) + layernorm(1):
        job()
    chk_s[...] = jnp.zeros_like(chk_s)
    for ref in (xf_s, ew_s, ex_s, aa0, aa1):
        ref[16:24, :128] = jnp.zeros((8, 128), u32)
    x_cp[2].start()
    w_cp[1].wait()
    wq = _cat([wqkvT_s[:64, :], _raw(wqkv_v[:, 128:512].T)], 0)
    wqkvT_s[64:256, :] = wq[64:]
    put_q(0, _cat([_dot(_up(wq[r:min(r + 64, D2)]), _up(xn_s[:, :256])) for r in range(0, D2, 64)], 0))
    w_cp[2].start()
    x_cp[1].wait()
    ex = [P(enc_x, t, c, r) for t in range(NT) for c in range(7) for r in range(7)]
    for jp in range(1, NC // 2):
        if jp == 4:
            x_cp[2].wait()
            for cp in w_cp[3:]:
                cp.start()
            w_cp[2].wait()
        pace = (_Pace(layernorm(jp + 1), 55 if jp == 3 else 48, [], [P(view, xf_s)], 14) if jp < 7 else
                _Pace(ex[:40], 54, [xf_s], [P(view, ex_s)], 14))
        put_q(jp, project(0, jp, pace))
        pace.finish()
    wqkvT_s[256:, :] = _raw(wqkv_v[:, 512:].T)
    pace = _Pace(ex[40:56], 54, [xf_s], [P(view, ex_s)], 14)
    for jp in range(NC // 2):
        if jp == 1:
            pace.restart(_merge(ex[56:], key_table(aa0, P(view, aa1), 1, 24), skip=10), 9 * 56,
                         [xf_s, aa1], [P(view, ex_s), P(view, aa0)])
        project(1, jp, pace)
    for jp in (0, 4):
        project(2, jp, pace)
    pace.finish()
    for cp in w_cp[3:]:
        cp.wait()

    @pl.loop(0, 2)
    def _(it):
        zero[0] = it >> 12
        lay_out_weights(it)
        aa1.at[A_K:][_part(it, 512), :] = head_k(1, _part(it, 512))
        d13 = ew_s.at[pl.ds(pl.multiple_of(O_W13 + it * 8, 8), 49 * (F4 // 2))]
        d2 = ew_s.at[pl.ds(pl.multiple_of(O_W2 + it * D8, 8), 53 * D4)]
        nq = NC // 2 * (DH + 1) * 8
        pace = _Pace(query_table(aa0.at[pl.ds(pl.multiple_of(A_QT + it * nq, 16), nq)],
                                 qf_s.at[0, :, _part(it, S // 2)], 1, NC // 4), 63, [], [P(view, aa0)], 14)
        for c in range(2 * NC):
            if c == 8:
                pace.restart([P(enc_w2, d2, n, r) for n in range(7) for r in range(7)]
                             + [P(enc_wo, d2, it, n) for n in range(7)], 127, [wd_s], [P(view, ew_s)])
            if c == 17:
                pace.restart([P(enc_w13, d13, n, r) for n in range(14) for r in range(7)], 236,
                             [wt_s], [P(view, ew_s)])
            if c in (12, 20, 26):
                project(2, 1 + (12, 20, 26).index(c), pace, it)
            sl = _part(2 * it + c // NC, T)
            s = _dot(_up(pace.lhs(view(k_s).at[0], c % NC * 64, 64, slice(0, 32))), _up(q_s[:16, sl]))
            pace.result(s)
            p_s[_part(c % NC, 64), sl] = _pk(jnp.exp2(s))
        pace.finish()

    @pl.loop(0, H // 2)
    def _(it):
        zero[0] = it >> 12
        pl.when(it > 0)(P(head_step, 2 * it, 0))
        head_step(2 * it + 1, 1)

    def finish(state):
        trip = state[0]
        pl.when(trip == 1)(exact_softmax)
        pl.loop(0, NT)(P(output_block, trip))
        trips = jnp.where(jnp.sum(chk_s[:8]) < 2.0 ** 120, 1, 2)
        pltpu.make_async_copy(o_v, oT_hbm, osem).wait()
        return trip + 1, trips
    lax.while_loop(lambda state: state[0] < state[1], finish, (np.int32(0), np.int32(1)))


@jax.jit
def pallas_parallel_sum__softmax_full_mha__glu_gated_swiglu__prompt_kernel(
    A_x: jax.Array,
    A_wqkv: jax.Array,
    A_wo: jax.Array,
    B_x: jax.Array,
    B_w1: jax.Array,
    B_w3: jax.Array,
    B_w2: jax.Array,
):
    del B_x
    assert A_x.shape == (1, S, D) and B_w1.shape == (D, F)
    V = pltpu.VMEM
    oT = pl.pallas_call(
        _kernel,
        name="mha_swiglu",
        in_specs=[pl.BlockSpec(memory_space=pl.ANY)] * 6,
        out_specs=pl.BlockSpec(memory_space=pl.ANY),
        out_shape=jax.ShapeDtypeStruct((D, S), bf16),
        scratch_shapes=[
            V((D, S), bf16), V((D, 3 * D), bf16), V((D, D), bf16), V((2, D, F), bf16), V((D, F), bf16),
            V((D, S), bf16),
            V((W_END, 256), u32),
            V((X_END, 256), u32),
            V((32 + NC // 2 * D, 256), u32),
            V((32 + 2 * F, 128), u32),
            V((32 + 5 * D, 128), u32),
            V((D2, S), u32),
            V((3 * D2, D), u32),
            V((28 * F4, 128), f32),
            V((H * 16, S), u32),
            V((H // 2, 64, S), f32),
            V((H // 4, S // 2, 128), u32),
            V((H * 16, S), u32),
            V((H // 2 + 1, 2 * DH, S), f32),
            V((32, 128), f32),
            V((S, S), u32),
            V((A_END, 128), u32), V((A_END, 128), u32),
            pltpu.SemaphoreType.DMA((3,)), pltpu.SemaphoreType.DMA((7,)), pltpu.SemaphoreType.DMA(()),
        ],
        compiler_params=pltpu.CompilerParams(vmem_limit_bytes=120 * 2**20),
    )(A_x.reshape(S, D).T, A_wqkv, A_wo, B_w1, B_w3, B_w2.T)
    return oT.T.reshape(1, S, D)
```

```python
import functools
import math

import jax
import jax.numpy as jnp
import numpy as np
from jax import lax
from jax.experimental import pallas as pl
from jax.experimental.pallas import tpu as pltpu

f32 = jnp.float32
bf16 = jnp.bfloat16
u32 = jnp.uint32
P = functools.partial

S, D, F, H = 2048, 448, 1792, 16
EPS = 1e-5
LOG2E = math.log2(math.e)

DH = D // H
D2, D4, D8, F4 = D // 2, D // 4, D // 8, F // 4
T = 512
NT = S // T
NC = S // 128
NG = 14
NV = 16 * NG
NM = S - NV
NW = -(-NV // 128)
DSTEP = 7
R = 64
AX = 512 - F4
AR = (D - 4 * AX) // 2
HEADROOM = 30.0

O_W13 = 32
O_W2 = O_W13 + 49 * (F4 // 2)
W_END = O_W2 + 53 * D4 + 80
O_XE = 32
X_END = O_XE + NT * 28 * D8
A_P = 32
A_K = A_P + 32
A_KT = A_K + S // 2
A_QT = A_KT + DH * NV + 16
A_KR = A_QT + NC * (DH + 1) * 8 + 16
A_END = A_KR + NW * (H // 2) * 64


def _pk(x):
    return pltpu.bitcast(x.astype(bf16), u32)


def _up(x):
    return pltpu.bitcast(x, bf16)


def _raw(x):
    return pltpu.bitcast(x, u32)


def _flt(x):
    return pltpu.bitcast(x, f32)


def _dot(a, b):
    return jnp.dot(a, b, preferred_element_type=f32)


def _cat(xs, axis):
    return jnp.concatenate(xs, axis=axis)


def _part(j, n):
    return slice(j * n, (j + 1) * n) if isinstance(j, int) else pl.ds(pl.multiple_of(j * n, n), n)


ENC_A = (((1, 0), (1, 3)), ((1, 2), (1, 3)), ((1, 0),), ((1, 3),), ((1, 0), (1, 1)), ((1, 2), (-1, 0)),
         ((1, 1), (-1, 3)))
ENC_B = (((1, 0), (1, 3)), ((1, 0),), ((1, 1), (-1, 3)), ((1, 2), (-1, 0)), ((1, 3),), ((1, 0), (1, 1)),
         ((1, 2), (1, 3)))
FLIP = (0, 1, 0, 0, 1, 1, 1)


def _comb(terms, get):
    x = get(terms[0][1])
    if len(terms) == 1:
        return x
    y = get(terms[1][1])
    return x + y if terms[1][0] > 0 else x - y


def _enc7(enc, r, get):
    o = [_comb(enc[r], lambda q: get(2 * (q // 2) + p // 2, 2 * (q % 2) + p % 2)) for p in range(4)]
    flip = FLIP[r] if enc is ENC_B else 0
    return [_comb(enc[s], lambda p: o[p ^ flip]) for s in range(7)]


def _dec(m):
    return [m[0] + m[3] - m[4] + m[6], m[2] + m[4], m[1] + m[3], m[0] - m[1] + m[2] + m[5]]


def _dec2(prod, extra=None):
    inner = [_dec([prod(r, s) for s in range(7)]) for r in range(7)]
    inner = [[m[p ^ f] for p in range(4)] for m, f in zip(inner, FLIP)]
    if extra:
        inner = [[x + y for x, y in zip(*e)] for e in zip(inner, extra)]
    out = [[None] * 4 for _ in range(4)]
    for i in range(2):
        for j in range(2):
            out[i][j], out[i][j + 2], out[i + 2][j], out[i + 2][j + 2] = _dec([m[2 * i + j] for m in inner])
    return out


class _Pace:
    def __init__(self, jobs, ticks, gate, tie, lag, lead=0):
        self.jobs, self.ticks, self.gate, self.tie, self.lag, self.lead = jobs, ticks, gate, tie, lag, lead
        self.pos, self.done, self.hist, self.last, self.later = 0, 0, [], -1, []

    def restart(self, jobs, ticks, gate, tie):
        self.run(len(self.jobs))
        self.jobs, self.ticks, self.gate, self.tie, self.lead, self.done = jobs, ticks, gate, tie, self.pos, 0

    def run(self, upto):
        while self.done < min(upto, len(self.jobs)):
            k = min(self.pos - self.lag, len(self.hist) - 1)
            if k > self.last:
                for ref in self.gate:
                    ref[:8, :128] = _raw(self.hist[k])
                self.last = k
            self.jobs[self.done]()
            self.done += 1

    def tick(self):
        done = self.done
        self.run((self.pos - self.lead) * len(self.jobs) // self.ticks)
        self.pos += 1
        due = [job for n, job in self.later if n == 0]
        self.later = [(n - 1, job) for n, job in self.later if n > 0]
        for job in due:
            job()
        return self.done > done or bool(due)

    def lhs(self, ref, o, n, lanes, tied=False):
        out = []
        for r in range(o, o + n, 8):
            ran = self.tick()
            x = ref[r:r + 8, lanes]
            for tie in self.tie if ran and not tied else []:
                x = x | tie()[16:24, :x.shape[1]]
            out.append(x)
        return _cat(out, 0)

    def result(self, y):
        self.hist += [y[r + 8:r + 16, -128:] for r in range(0, y.shape[0], 16)]

    def finish(self):
        self.run(len(self.jobs))
        for _, job in self.later:
            job()
        self.later = []


def _merge(before, main, after, skip):
    def share(lists, n):
        for lst in lists:
            for job in lst[max(n - skip, 0) * len(lst) // (len(main) - skip):
                           max(n + 1 - skip, 0) * len(lst) // (len(main) - skip)]:
                job()

    def joined(n):
        share(before, n)
        main[n]()
        share(after, n)
    return [P(joined, n) for n in range(len(main))]


def _kernel(xT_hbm, wqkv_hbm, wo_hbm, w1_hbm, w3_hbm, w2T_hbm, oT_hbm,
            x_v, wqkv_v, wo_v, w13_v, w2T_v, o_v,
            ew_s, ex_s, xf_s, wt_s, wd_s, xn_s, wqkvT_s, h_s, q_s, qf_s, k_s, v_s, a_s, chk_s, p_s, aa0, aa1,
            xsem, wsem, osem):
    x_cuts = (0, 512, 1280, S)
    x_cp = [pltpu.make_async_copy(xT_hbm.at[:, a:b], x_v.at[:, a:b], xsem.at[n])
            for n, (a, b) in enumerate(zip(x_cuts, x_cuts[1:]))]
    w_cuts = (0, 128, 512, 3 * D)
    w_cp = [pltpu.make_async_copy(src, dst, wsem.at[n]) for n, (src, dst) in enumerate(
        [(wqkv_hbm.at[:, a:b], wqkv_v.at[:, a:b]) for a, b in zip(w_cuts, w_cuts[1:])]
        + [(w1_hbm, w13_v.at[0]), (wo_hbm, wo_v), (w2T_hbm, w2T_v), (w3_hbm, w13_v.at[1])])]
    x_cp[0].start()
    w_cp[0].start()
    w_cp[1].start()

    zero = [lax.fori_loop(0, 2, lambda i, c: (c + i) >> 12, np.int32(0))]
    views = [0]

    def view(ref, start=0, size=None):
        views[0] += 1
        return ref.at[pl.ds(pl.multiple_of(zero[0] * (32 * views[0]) + start, 32), size or ref.shape[0])]

    row = lax.broadcasted_iota(jnp.int32, (32, 256), 0)

    def window(y, h, first, rest):
        off = 4 * (h % 2)
        w = y[h * DH - off:h * DH - off + 32]
        b = slice(0, 8) if off else slice(24, 32)
        fill = jnp.where(row[b] == (0 if off else DH), first, rest)
        e = jnp.where((row[b] >= off) & (row[b] < off + DH), w[b], fill)
        return _cat([e, w[8:]] if off else [w[:24], e], 0)

    def layernorm(jp):
        stat = {}

        def rows(c):
            return view(x_v)[_part(c, 32), _part(jp, 256)].astype(f32)

        def total(x, n, c):
            x = x[0:8] + x[8:16] + (x[16:24] + x[24:32])
            stat[n] = x if c == 0 else stat[n] + x
            if c == D // 32 - 1:
                stat[n] = jnp.sum(stat[n], axis=0, keepdims=True) * (1.0 / D)
            xf_s[8:16, :] = _raw(jnp.broadcast_to(stat[n], (8, 256)))

        def mean(c):
            total(rows(c), 0, c)

        def var(c):
            xc = rows(c) - stat[0]
            total(xc * xc, 1, c)

        def put(c):
            xn = (rows(c) - stat[0]) * lax.rsqrt(stat[1] + EPS)
            xf_s[32 + jp * D + c * 32:32 + jp * D + (c + 1) * 32, :] = _raw(xn)
            xn_s[_part(c, 16), _part(jp, 256)] = _pk(xn)
        return [P(f, c) for f in (mean, var, put) for c in range(D // 32)]

    def put_q(jp, q):
        qf_s[:, :2 * DH, _part(jp, 256)] = (q * (DH ** -0.5 * LOG2E)).reshape(H // 2, 2 * DH, 256)

    def put_qk(jp, g, k):
        sl = _part(jp, 256)

        def head(n):
            h = 4 * g + n
            q = qf_s[h // 2, :2 * DH, sl]
            own = jnp.sum(window(q * k[_part(n // 2, 2 * DH)], h % 2, 0.0, 0.0), axis=0, keepdims=True)
            shift = (-HEADROOM - own).astype(bf16).astype(f32)
            qf_s[h // 2, 2 * DH + h % 2:2 * DH + h % 2 + 1, sl] = shift
            q_s[_part(h, 16), sl] = _pk(window(q, h % 2, shift, 0.0))
            ex_s[8:16, :] = q_s[_part(2 * h + 1 - h % 2, 8), sl]

        def keys(n):
            kT = _raw(_cat([window(k, h, 1.0, 0.0) for h in range(4)], 0)[:, _part(n, 128)].astype(bf16).T)
            k_s[g, _part((jp + 7) % 8 * 2 + n, 64), :] = kT
            ex_s[8:16, :128] = kT[-8:]

        def key_rows(w, n):
            o = A_KR + (w * (H // 2) + 2 * g + n) * 64
            for ref in (aa0, aa1):
                ref[o:o + 2 * DH, :] = _raw(pltpu.roll(k, NV % 256, 1)[_part(n, 2 * DH), _part(w, 128)])
        return ([(10 + 2 * n, P(head, n)) for n in range(4)] + [(30 + 6 * n, P(keys, n)) for n in range(2)]
                + [(22 + 2 * n + w, P(key_rows, w, n)) for n in range(2) for w in range(NW) if jp == 0])

    def project(part, jp, pace, half=0):
        ys = []

        def rhs(n):
            return _up(view(xn_s).at[:, _part(half + jp // 4, S // 2)][:, _part(jp % 4 * 2 + n, 128)])
        xn = [rhs(n) for n in range(2)] if part == 0 else None
        for g in range(4):
            o = part * D2 + g * D8
            y = []
            for n in range(2):
                src = view(wqkvT_s)
                lhs = _cat([pace.lhs(src, o, D8, slice(0, 128)), src[o:o + D8, 128:]], 1)
                y.append(_dot(_up(lhs), xn[n] if xn else rhs(n)))
                pace.result(y[-1])
            ys.append(_cat(y, 1))
            if part == 1:
                pace.later += put_qk(jp, g, ys[-1])
            if part == 2:
                for n in range(4):
                    v_s[_part(4 * g + n, 16), _part((4 * half + jp + 7) & 7, 256)] = _pk(window(ys[-1], n, 1.0, 1.0))
        return _cat(ys, 0)

    def enc_x(t, c, r):
        src = view(xf_s)

        def get(i, j):
            o = 32 + (2 * t + j // 2) * D + i * D4 + c * 16
            return _flt(src[o:o + 16, _part(j % 2, 128)])
        e = _enc7(ENC_B, r, get)
        for p in range(4):
            o = O_XE + ((t * 7 + r) * 4 + p) * D8 + c * 8
            ex_s[o:o + 8, :] = _pk(_cat([e[2 * p], e[min(2 * p + 1, 6)]], 1))

    def enc_w(src, where, dst, stride, o, r):
        src = view(src)
        for s, e in enumerate(_enc7(ENC_A, r, lambda i, j: _up(
                _cat([src[a:a + 8, :] for a in where(i, j)], 1)).astype(f32))):
            dst[o + (7 * r + s) * stride:o + (7 * r + s) * stride + 8, :] = _pk(e)

    def enc_w13(dst, n, r):
        enc_w(wt_s, lambda i, j: [32 + j * (F // 2) + a + (192 * i + 16 * n if n < 12 else 576 + 32 * i + 16 * n)
                                  for a in (0, 8)], dst, F4 // 2, n * 16, r)

    def enc_w2(dst, c, r):
        enc_w(wd_s, lambda i, j: [32 + (2 * j + a) * D2 + i * D8 + c * 8 for a in range(2)], dst, D4, c * 8, r)

    def enc_wo(dst, m, c):
        src = view(wd_s).at[pl.ds(pl.multiple_of(32 + 4 * D + m * D8, 8), D - D8)]
        q = [_up(src[o + c * 8:o + c * 8 + 8, :]).astype(f32) for o in (0, D2, D4, D2 + D4)]
        for p in range(4):
            o = (49 + p) * D4 + c * 8
            dst[o:o + 8, :] = _pk(_cat([_comb(ENC_A[r], lambda n: q[n]) for r in (2 * p, min(2 * p + 1, 6))], 1))

    def wo_t(r0, n):
        w = _cat([wo_v[r0:r0 + n, :], jnp.zeros((n, 512 - D), bf16)], 1)
        if n % 128:
            w = _cat([w, jnp.zeros((-n % 128, 512), bf16)], 0)
        return _raw(w.T)[:D2]

    def lay_out_weights(m):
        woT = wo_t(0, 4 * AX)
        for n in range(2):
            wd_s[32 + 4 * D + n * D2:32 + 4 * D + (n + 1) * D2, :] = wo_t(4 * AX + n * AR, AR)
        lane = lax.broadcasted_iota(jnp.int32, (D2, 128), 1)
        for j in range(4):
            o = 32 + 2 * j * D2
            wd_s[o:o + D2, :] = _raw(w2T_v[:, pl.ds(pl.multiple_of(384 * j + 256 * m, 128), 128)])
            b = _raw(w2T_v[:, _part(12 + j // 2, 128)])
            wo = woT[:, _part(j // 2, 128)]
            b = jnp.where(lane < 64, b, wo) if j % 2 == 0 else pltpu.roll(jnp.where(lane < 64, wo, b), 64, 1)
            wd_s[o + D2:o + D, :] = jnp.where(m == 0, _raw(w2T_v[:, _part(3 * j + 1, 128)]), b)
        for j in range(4):
            w = _cat([w13_v[m, _part(j, D4), :], jnp.zeros((128 - D4, F), bf16)], 0)
            wt_s[32 + j * (F // 2):32 + (j + 1) * (F // 2), :] = _raw(w.T)

    def key_table(dst, src, par, ahead):
        val = {}

        def start(d, w):
            r, n = par * DH + d, min(128, NV - 128 * w)
            o = A_KR + w * (H // 2) * 64 + r // 8 * 8
            val[d, w] = jnp.broadcast_to(src()[o:o + 8, :n][r % 8:r % 8 + 1], (128, n)).T

        def put(d, g):
            o = A_KT + (g * DH + d) * 16
            dst[o:o + 16, :] = val[d, g // 8][_part(g % 8, 16)]
        puts = [(d, g) for d in range(DH) for g in range(NG)]
        jobs = []
        for n in range(len(puts) + ahead):
            if n < len(puts) and puts[n][1] % 8 == 0:
                jobs.append(P(start, puts[n][0], puts[n][1] // 8))
            if n >= ahead:
                jobs.append(P(put, *puts[n - ahead]))
        return jobs

    def query_table(dst, src, par, pairs):
        def put(j, d):
            r = par * DH + d if d < DH else 2 * DH + par
            dst[_part(j * (DH + 1) + d, 16), :] = _raw(_cat(
                [jnp.broadcast_to(src[r:r + 1, _part(2 * j + n, 128)], (8, 128)) for n in range(2)], 0))
        return [P(put, j, d) for j in range(pairs) for d in range(DH + 1)]

    def head_k(h, rows):
        return pltpu.roll(k_s[h >> 2, rows, :], (-h & 3) * 32, 1)

    def put_k(dst, h, r):
        dst[A_K + r:A_K + r + 8, :] = head_k(h, slice(r, r + 8))

    def head_rows(ref, h):
        return ref.at[_part(h, 16)]

    def put_a(h, par, sl, acc):
        inv = pltpu.reciprocal(acc[0:1] if par else acc[31:32], approx=True)
        a_s[h >> 1, _part(par, DH), sl] = (acc * inv)[4 * par:4 * par + DH]
        return inv

    def weigh(h, par, t, j, c, acc, pace, dst):
        p = p_s.at[:, _part(t, T)][_part(par * 4 + c, 256), _part(j, 128)]
        src = head_rows(view(v_s), h)
        v = _cat([pace.lhs(src, 0, 16, _part(4 * c, 128)), src[:, c * 512 + 128:(c + 1) * 512]], 1)
        d = _dot(_up(v), _up(p))
        acc = d if c == 0 else d + acc
        pace.result(acc)
        if c == 3:
            inv = put_a(dst, par, _part(4 * t + j, 128), acc)
            a = jnp.abs(acc)
            chk_s[:8] += a[0:8] + a[8:16] + (a[16:24] + a[24:32]) + inv * 2.0 ** 80
        return acc

    def head_step(h, par):
        cur, oth = (aa0, aa1) if par == 0 else (aa1, aa0)
        hn = jnp.minimum(h + 1, H - 1)
        part = []

        def unit(jp, g, d0):
            src = view(oth)
            oq, ok = A_QT + jp * (DH + 1) * 16, A_KT + g * DH * 16
            if d0 == 0:
                q = _flt(src[oq + DH * 16:oq + (DH + 1) * 16, :])
                part[:] = [_cat([q[o:o + 8]] * 2, 0) for o in (0, 8)]
            k = _flt(src[ok + d0 * 16:ok + (d0 + DSTEP) * 16, :])
            q = _flt(src[oq + d0 * 16:oq + (d0 + DSTEP) * 16, :])
            for o in range(0, DSTEP * 16, 16):
                part[:] = [a + k[o:o + 16] * _cat([q[o + n:o + n + 8]] * 2, 0) for a, n in zip(part, (0, 8))]
            cur[A_P:A_P + 32, :] = _raw(_cat(part, 0))
            if d0 + DSTEP == DH:
                o = (par * S + NM) // 2 + g * 8
                p_s[o:o + 8, _part(jp, 256)] = _pk(jnp.exp2(_cat(part, 1)))

        jobs = _merge([[P(put_k, oth, hn, r) for r in range(0, NM // 2, 8)]],
                      [P(unit, jp, g, d0) for jp in range(NC // 2) for g in range(NG) for d0 in range(0, DH, DSTEP)],
                      [key_table(cur, P(view, oth, (hn >> 1) * 64, A_END - (H // 2 - 1) * 64), 1 - par, 12),
                       query_table(cur.at[A_QT:], qf_s.at[hn >> 1], 1 - par, NC // 2)], 2)
        pace = _Pace(jobs, NT * (NM // 16 + 2 * NC) - 6, [oth], [P(view, cur)], 13, 8)
        acc = None
        for t in range(NT):
            for c in range(NC):
                a, b = NM // 16 * c // NC * 8, NM // 16 * (c + 1) // NC * 8
                last = t == NT - 1 and c == NC - 1
                if last:
                    weigh(h - 1, 1 - par, t, c // 4, c % 4, acc, pace, h - 1)
                k = pace.lhs(view(cur) if t + c else cur, A_K + a, b - a, slice(0, 32), tied=True)
                s = _dot(_up(k), _up(head_rows(q_s, h)[:, _part(t, T)]))
                pace.result(s)
                if not last:
                    acc = weigh(h - 1, 1 - par, t, c // 4, c % 4, acc, pace, h - 1)
                p_s[par * S // 2 + a:par * S // 2 + b, _part(t, T)] = _pk(jnp.exp2(s))
        pace.finish()

    def exact_softmax():
        @pl.loop(0, H * NC)
        def _(n):
            h, sl = n // NC, _part(n % NC, 128)
            q = _up(head_rows(q_s, h)[:, sl]).astype(f32)
            q = jnp.where(row[:, :128] == (1 - h % 2) * DH, 0.0, q).astype(bf16)

            def scores(c, m):
                s = _dot(_up(head_k(h, _part(c, 256))[:, :32]), q)
                h_s[_part(c, 512), :] = s
                return jnp.maximum(m, jnp.max(s, axis=0, keepdims=True))
            m = lax.fori_loop(0, 4, scores, jnp.full((1, 128), -jnp.inf, f32))
            acc = lax.fori_loop(0, 4, lambda c, acc: acc + _dot(
                _up(head_rows(v_s, h)[:, _part(c, 512)]), jnp.exp2(h_s[_part(c, 512), :] - m).astype(bf16)),
                jnp.zeros((32, 128), f32))
            for par in range(2):
                @pl.when(h % 2 == par)
                def _():
                    put_a(h, par, sl, acc)

    def a_rows(src, r0, r1, sl):
        n = 2 * DH
        return _cat([src[g, max(r0 - g * n, 0):min(r1 - g * n, n), sl] for g in range(r0 // n, -(-r1 // n))], 0)

    def output_block(trip, t):
        zero[0] = t >> 12
        last_head = [0, None]
        for c in range(F4 // R):
            xe = view(ex_s, t * 28 * D8, O_XE + 28 * D8)

            def up(r, s):
                if (49 * c + 7 * r + s) % 8 == 4 and last_head[0] < 16:
                    last_head[1] = weigh(H - 1, 1, t, last_head[0] // 4, last_head[0] % 4, last_head[1],
                                         _Pace([], 1, [], [], 0), H - 1 + trip * 2)
                    last_head[0] += 1
                o = O_W13 + (7 * r + s) * (F4 // 2) + c * R // 2
                w = ew_s[o:o + R // 2, :]
                lhs = _cat([w[_part(n // 2 * 2 + m, 8), n % 2 * 128:n % 2 * 128 + D4]
                            for m in range(2) for n in range(R // 16)], 0)
                o = O_XE + (4 * r + s // 2) * D8
                return _dot(_up(lhs), _up(xe[o:o + D8, _part(s % 2, 128)]))
            hid = [[y[:R] * y[R:] * pltpu.reciprocal(1.0 + jnp.exp2(y[:R] * -LOG2E), approx=True) for y in ys]
                   for ys in _dec2(up)]
            for p in range(4):
                for r in range(7):
                    h_s[(4 * r + p) * F4 + c * R:(4 * r + p) * F4 + (c + 1) * R, :] = _comb(
                        ENC_B[r], lambda q: hid[2 * (q // 2) + p // 2][2 * (q % 2) + p % 2])

        av = view(a_s).at[:, :, _part(t, T)]
        extra = []
        for r in range(7):
            e = _comb(ENC_B[r], lambda q: a_rows(av, 4 * AX + q // 2 * AR, 4 * AX + (q // 2 + 1) * AR,
                                                 _part(q % 2, 256)))
            o = O_W2 + (49 + r // 2) * D4
            extra.append([_dot(_up(ew_s[o + p // 2 * D8:o + (p // 2 + 1) * D8, r % 2 * 128:r % 2 * 128 + AR]),
                               e[:, _part(p % 2, 128)].astype(bf16)) for p in range(4)])

        def down(r, s):
            hv, av = view(h_s), view(a_s).at[:, :, _part(t, T)]

            def a_blk(p, q):
                i, j = (2 * (q // 2) + p // 2) ^ 1, 2 * (q % 2) + p % 2
                return a_rows(av, i * AX, (i + 1) * AX, _part(j, 128))
            e = _comb(ENC_B[s], lambda p: _cat([hv[_part(4 * r + (p ^ FLIP[r]), F4), :],
                                                _comb(ENC_B[r], P(a_blk, p ^ FLIP[r]))], 0))
            o = O_W2 + (7 * r + s) * D4
            return _dot(_up(_cat([ew_s[o:o + D8, :], ew_s[o + D8:o + D4, :]], 1)), e.astype(bf16))
        y = _dec2(down, extra)
        for q in (2, 1, 3, 0):
            rows, lanes = _part(q // 2, D2), _part(2 * t + q % 2, 256)
            yq = _cat([_cat(y[q // 2 * 2 + n][_part(q % 2, 2)], 1) for n in range(2)], 0)
            view(o_v)[rows, lanes] = (x_v.at[:, _part(t, T)][rows, _part(q % 2, 256)].astype(f32) + yq).astype(bf16)
            pltpu.make_async_copy(o_v.at[rows, lanes], oT_hbm.at[rows, lanes], osem).start()

    x_cp[0].wait()
    x_cp[1].start()
    w_cp[0].wait()
    wqkvT_s[:64, :] = _raw(wqkv_v[:, :128].T)
    for job in layernorm(0) + layernorm(1):
        job()
    chk_s[...] = jnp.zeros_like(chk_s)
    for ref in (xf_s, ew_s, ex_s, aa0, aa1):
        ref[16:24, :128] = jnp.zeros((8, 128), u32)
    x_cp[2].start()
    w_cp[1].wait()
    wq = _cat([wqkvT_s[:64, :], _raw(wqkv_v[:, 128:512].T)], 0)
    wqkvT_s[64:256, :] = wq[64:]
    put_q(0, _cat([_dot(_up(wq[r:min(r + 64, D2)]), _up(xn_s[:, :256])) for r in range(0, D2, 64)], 0))
    w_cp[2].start()
    x_cp[1].wait()
    ex = [P(enc_x, t, c, r) for t in range(NT) for c in range(7) for r in range(7)]
    for jp in range(1, NC // 2):
        if jp == 4:
            x_cp[2].wait()
            for cp in w_cp[3:]:
                cp.start()
            w_cp[2].wait()
        pace = (_Pace(layernorm(jp + 1), 55 if jp == 3 else 48, [], [P(view, xf_s)], 14) if jp < 7 else
                _Pace(ex[:32], 54, [xf_s], [P(view, ex_s)], 15))
        put_q(jp, project(0, jp, pace))
        pace.finish()
    wqkvT_s[256:, :] = _raw(wqkv_v[:, 512:].T)
    pace = _Pace(ex[32:42], 54, [xf_s], [P(view, ex_s)], 15)
    for jp in range(NC // 2):
        if jp == 1:
            pace.restart(_merge([key_table(aa0, P(view, aa1), 1, 24)], ex[42:], [], 10), 9 * 56,
                         [xf_s, aa1], [P(view, ex_s), P(view, aa0)])
        project(1, jp, pace)
    for jp in (0, 4):
        project(2, jp, pace)
    pace.finish()
    for cp in w_cp[3:]:
        cp.wait()

    @pl.loop(0, 2)
    def _(it):
        zero[0] = it >> 12
        lay_out_weights(it)
        aa1.at[A_K:][_part(it, 512), :] = head_k(1, _part(it, 512))
        d13 = ew_s.at[pl.ds(pl.multiple_of(O_W13 + it * 8, 8), 49 * (F4 // 2))]
        d2 = ew_s.at[pl.ds(pl.multiple_of(O_W2 + it * D8, 8), 53 * D4)]
        nq = NC // 2 * (DH + 1) * 8
        pace = _Pace(query_table(aa0.at[pl.ds(pl.multiple_of(A_QT + it * nq, 16), nq)],
                                 qf_s.at[0, :, _part(it, S // 2)], 1, NC // 4), 63, [], [P(view, aa0)], 14)
        for c in range(2 * NC):
            if c == 8:
                pace.restart([P(enc_w2, d2, n, r) for n in range(7) for r in range(7)]
                             + [P(enc_wo, d2, it, n) for n in range(7)], 143, [wd_s], [P(view, ew_s)])
            if c == 19:
                pace.restart([P(enc_w13, d13, n, r) for n in range(14) for r in range(7)], 220,
                             [wt_s], [P(view, ew_s)])
            if c in (12, 21, 27):
                project(2, 1 + (12, 21, 27).index(c), pace, it)
            sl = _part(2 * it + c // NC, T)
            s = _dot(_up(pace.lhs(view(k_s).at[0], c % NC * 64, 64, slice(0, 32))), _up(q_s[:16, sl]))
            pace.result(s)
            p_s[_part(c % NC, 64), sl] = _pk(jnp.exp2(s))
        pace.finish()

    @pl.loop(0, H // 2)
    def _(it):
        zero[0] = it >> 12
        pl.when(it > 0)(P(head_step, 2 * it, 0))
        head_step(2 * it + 1, 1)

    def finish(state):
        trip = state[0]
        pl.when(trip == 1)(exact_softmax)
        pl.loop(0, NT)(P(output_block, trip))
        trips = jnp.where(jnp.sum(chk_s[:8]) < 2.0 ** 120, 1, 2)
        pltpu.make_async_copy(o_v, oT_hbm, osem).wait()
        return trip + 1, trips
    lax.while_loop(lambda state: state[0] < state[1], finish, (np.int32(0), np.int32(1)))


@jax.jit
def pallas_parallel_sum__softmax_full_mha__glu_gated_swiglu__prompt_kernel(
    A_x: jax.Array,
    A_wqkv: jax.Array,
    A_wo: jax.Array,
    B_x: jax.Array,
    B_w1: jax.Array,
    B_w3: jax.Array,
    B_w2: jax.Array,
):
    del B_x
    assert A_x.shape == (1, S, D) and B_w1.shape == (D, F)
    V = pltpu.VMEM
    oT = pl.pallas_call(
        _kernel,
        name="mha_swiglu",
        in_specs=[pl.BlockSpec(memory_space=pl.ANY)] * 6,
        out_specs=pl.BlockSpec(memory_space=pl.ANY),
        out_shape=jax.ShapeDtypeStruct((D, S), bf16),
        scratch_shapes=[
            V((D, S), bf16), V((D, 3 * D), bf16), V((D, D), bf16), V((2, D, F), bf16), V((D, F), bf16),
            V((D, S), bf16),
            V((W_END, 256), u32),
            V((X_END, 256), u32),
            V((32 + NC // 2 * D, 256), u32),
            V((32 + 2 * F, 128), u32),
            V((32 + 5 * D, 128), u32),
            V((D2, S), u32),
            V((3 * D2, D), u32),
            V((28 * F4, 128), f32),
            V((H * 16, S), u32),
            V((H // 2, 64, S), f32),
            V((H // 4, S // 2, 128), u32),
            V((H * 16, S), u32),
            V((H // 2 + 1, 2 * DH, S), f32),
            V((32, 128), f32),
            V((S, S), u32),
            V((A_END, 128), u32), V((A_END, 128), u32),
            pltpu.SemaphoreType.DMA((3,)), pltpu.SemaphoreType.DMA((7,)), pltpu.SemaphoreType.DMA(()),
        ],
        compiler_params=pltpu.CompilerParams(vmem_limit_bytes=120 * 2**20),
    )(A_x.reshape(S, D).T, A_wqkv, A_wo, B_w1, B_w3, B_w2.T)
    return oT.T.reshape(1, S, D)
```
